```python
import jax
import jax.numpy as jnp

def _softmax(x, axis=-1):
    return jax.nn.softmax(x, axis=axis)
def _gelu(x):
    return jax.nn.gelu(x, approximate=True)
def _silu(x):
    return jax.nn.silu(x)
def _sigmoid(x):
    return jax.nn.sigmoid(x)
def _layernorm(x, axis=-1, eps=1e-5):
    m = jnp.mean(x, axis=axis, keepdims=True)
    v = jnp.var(x, axis=axis, keepdims=True)
    return (x - m) / jnp.sqrt(v + eps)
def _scatter_add(tgt, idx, src, axis=0):
    return tgt.at[idx].add(src)
def _segment_sum(src, seg, n):
    return jax.ops.segment_sum(src, seg, n)
class _Rng:
    def __init__(self, key):
        self._k = key
    def _next(self):
        self._k, sub = jax.random.split(self._k)
        return sub
    def normal(self, shape):
        return jax.random.normal(self._next(), shape, dtype=jnp.bfloat16)
    def randint(self, lo, hi, shape):
        return jax.random.randint(self._next(), shape, lo, hi, dtype=jnp.int32)
    def uniform(self, shape, lo=0.0, hi=1.0):
        return jax.random.uniform(self._next(), shape, jnp.bfloat16, lo, hi)
    def permutation(self, n):
        return jax.random.permutation(self._next(), n)


kernel_name = 'standalone__cross_network_dcn__recsys'

def setup_inputs():
    _rng = _Rng(jax.random.key(int.from_bytes(__import__("os").urandom(4), "little")))
    _w = (lambda a: (lambda t: t.astype(jnp.bfloat16) if jnp.issubdtype(t.dtype, jnp.floating) else t)(jnp.asarray(a)))
    B, F, D, L = 16384, 100, 16, 6
    Din = min(F * D, 1024)
    return {
        "x0": _w((lambda *s: _rng.normal(s) * 0.05)(B, Din)),
        "ws": _w((lambda *s: _rng.normal(s) * 0.05)(L, Din, Din) * (Din ** -0.5)),
        "bs": _w((lambda *s: _rng.normal(s) * 0.05)(L, Din) * 0.01),
    }

def reference(x0, ws, bs):
    x = x0
    L = ws.shape[0]
    for l in range(L):
        proj = jnp.einsum('bd,de->be', x, ws[l]) + bs[l]
        x = x0 * proj + x
    return x
```

```python
import jax
import jax.numpy as jnp
import jax.experimental.pallas as pl
import jax.experimental.pallas.tpu as pltpu

TM = 512


def _kernel(x0_ref, w_ref, b_ref, o_ref):
    L = w_ref.shape[0]
    x = x0_ref[...]
    for l in range(L):
        p = jnp.dot(x, w_ref[l], preferred_element_type=jnp.float32)
        p = p + b_ref[l:l + 1, :].astype(jnp.float32)
        y = x0_ref[...].astype(jnp.float32) * p + x.astype(jnp.float32)
        x = y.astype(o_ref.dtype)
    o_ref[...] = x


@jax.jit
def pallas_standalone__cross_network_dcn__recsys_kernel(x0, ws, bs):
    B, D = x0.shape
    L = ws.shape[0]
    return pl.pallas_call(
        _kernel,
        grid=(B // TM,),
        in_specs=[
            pl.BlockSpec((TM, D), lambda i: (i, 0)),
            pl.BlockSpec((L, D, D), lambda i: (0, 0, 0), pipeline_mode=pl.Buffered(1)),
            pl.BlockSpec((L, D), lambda i: (0, 0), pipeline_mode=pl.Buffered(1)),
        ],
        out_specs=pl.BlockSpec((TM, D), lambda i: (i, 0)),
        out_shape=jax.ShapeDtypeStruct((B, D), x0.dtype),
        compiler_params=pltpu.CompilerParams(
            dimension_semantics=("arbitrary",), vmem_limit_bytes=100 * 1024 * 1024),
    )(x0, ws, bs)
```

```python
import jax
import jax.numpy as jnp
import jax.experimental.pallas as pl
import jax.experimental.pallas.tpu as pltpu

f32 = jnp.float32
bf16 = jnp.bfloat16

A_TERMS = {1: [(1, 0), (1, 3)], 2: [(1, 2), (1, 3)], 3: [(1, 0)], 4: [(1, 3)],
           5: [(1, 0), (1, 1)], 6: [(1, 2), (-1, 0)], 7: [(1, 1), (-1, 3)]}
B_TERMS = {1: [(1, 0), (1, 3)], 2: [(-1, 0)], 3: [(1, 1), (-1, 3)], 4: [(1, 2), (-1, 0)],
           5: [(-1, 3)], 6: [(1, 0), (1, 1)], 7: [(1, 2), (1, 3)]}
C_TERMS = {1: [(1, 0), (1, 3)], 2: [(-1, 2), (1, 3)], 3: [(1, 1), (1, 3)], 4: [(1, 0), (1, 2)],
           5: [(1, 0), (-1, 1)], 6: [(1, 3)], 7: [(1, 0)]}
C_COUNT = (4, 2, 2, 4)
OUTER = ((3, 5, 6, 1, 2, 4, 7), (4, 2, 7, 1, 5, 3, 6))
INNER = (7, 4, 2, 1, 6, 3, 5)
BLOCKS = [(q, s) for q in range(4) for s in range(4)]


def rc(q, s):
    return (q // 2) * 2 + s // 2, (q % 2) * 2 + s % 2


def addsub(u, v, sg):
    return u + v if sg > 0 else u - v


def comb(terms, get):
    u = get(terms[0][1])
    if len(terms) == 1:
        return u if terms[0][0] > 0 else -u
    return addsub(u, get(terms[1][1]), terms[1][0])


def lhs(m1, m2, X):
    t1, t2 = A_TERMS[m1], A_TERMS[m2]
    if len(t1) == 1 or len(t2) == 1:
        return comb(t2, lambda s: comb(t1, lambda q: X(q, s)))
    (_, q0), (g1, q1) = t1
    (_, s0), (g2, s1) = t2
    u = addsub(X(q0, s0), X(q1, s1), g1 * g2)
    if g1 < 0 < g2:
        return u + (X(q0, s1) - X(q1, s0))
    return addsub(u, addsub(X(q1, s0), X(q0, s1), g1 * g2), g1)


def layer(parity, X, X0, W, bias, emit, inner=INNER):
    pend = {k: [] for k in BLOCKS}
    cnt = {(q, s): C_COUNT[q] for q, s in BLOCKS}
    for m1 in OUTER[parity]:
        acc = [None] * 4
        left = list(C_COUNT)
        for m2 in inner:
            p = jnp.dot(lhs(m1, m2, X).astype(bf16), W((m1 - 1) * 7 + m2 - 1), preferred_element_type=f32)
            for sg, s in C_TERMS[m2]:
                acc[s] = p if acc[s] is None else addsub(acc[s], p, sg)
                left[s] -= 1
                if left[s]:
                    continue
                for sg1, q in C_TERMS[m1]:
                    lst = sorted(pend[q, s] + [(sg1, acc[s])], key=lambda e: -e[0])
                    cnt[q, s] -= 1
                    if (cnt[q, s] == 0 or m1 != 1) and lst[0][0] > 0:
                        tot = lst[0][1]
                        for sg2, v in lst[1:]:
                            tot = addsub(tot, v, sg2)
                        lst = [(1, tot)]
                    pend[q, s] = lst
                    if cnt[q, s] == 0:
                        emit(q, s, X0(q, s) * (lst[0][1] + bias(q, s)) + X(q, s))


def build(tm=256, T=2, vmem=100, u32=True, overlap=True, flags=None):
    qm = tm // 4
    PR = 16

    def kern(x0_ref, w_hbm, b_ref, o_ref, s0_ref, s1_ref, wbuf, xa_ref, xb_ref, sem):
        L, D, _ = w_hbm.shape
        h = D // 4
        s_refs = (s0_ref, s1_ref)

        def blk(ref, q, s):
            r, c = rc(q, s)
            return ref.at[r * qm:(r + 1) * qm, c * h:(c + 1) * h]

        def wload(par, lp):
            if u32:
                return lambda k: pltpu.bitcast(s_refs[par][lp, k], bf16)
            return lambda k: s_refs[par][lp, k]

        def prep(par, lp, r0):
            b = {}
            for q, s in BLOCKS:
                r, c = rc(q, s)
                b[q, s] = wbuf[par, pl.ds(r * h + r0, PR), c * h:(c + 1) * h].astype(f32)
            for m1 in range(1, 8):
                sub = [comb(B_TERMS[m1], lambda q: b[q, s]) for s in range(4)]
                for m2 in range(1, 8):
                    v = comb(B_TERMS[m2], lambda s: sub[s]).astype(bf16)
                    k = (m1 - 1) * 7 + m2 - 1
                    if u32:
                        s_refs[par][lp, k, pl.ds(pl.multiple_of(r0 // 2, PR // 2), PR // 2), :] = pltpu.bitcast(v, jnp.uint32)
                    else:
                        s_refs[par][lp, k, pl.ds(r0, PR), :] = v

        def prep_all(par, lp):
            def body(i, c):
                prep(par, lp, pl.multiple_of(i * PR, PR))
                return c
            jax.lax.fori_loop(0, h // PR, body, 0)

        def wcopy(l, par):
            return pltpu.make_async_copy(w_hbm.at[l], wbuf.at[par], sem.at[par])

        @pl.when(pl.program_id(0) == 0)
        def _first():
            wcopy(0, 0).start()
            xa_ref[...] = x0_ref[...].astype(f32)
            wcopy(0, 0).wait()
            wcopy(1, 1).start()
            prep_all(0, 0)

            def phase(par, lp, src, dst):
                l = 2 * lp + par
                if overlap:
                    @pl.when(l + 1 < L)
                    def _():
                        wcopy(l + 1, 1 - par).wait()
                @pl.when(l + 2 < L)
                def _():
                    wcopy(l + 2, par).start()

                def body(t, c):
                    rows = pl.ds(pl.multiple_of(t * tm, tm), tm)
                    x0t, st, dt = x0_ref.at[rows], src.at[rows], dst.at[rows]
                    def emit(q, s, y):
                        blk(dt, q, s)[...] = y
                    layer(par, lambda q, s: blk(st, q, s)[...], lambda q, s: blk(x0t, q, s)[...].astype(f32),
                          wload(par, lp),
                          lambda q, s: b_ref[lp, par:par + 1, rc(q, s)[1] * h:(rc(q, s)[1] + 1) * h].astype(f32), emit)
                    if overlap:
                        n = h // PR // T
                        for i in range(n):
                            prep(1 - par, lp + par, pl.multiple_of((t * n + i) * PR, PR))
                    return c
                jax.lax.fori_loop(0, T, body, 0)
                if not overlap:
                    @pl.when(l + 1 < L)
                    def _():
                        wcopy(l + 1, 1 - par).wait()
                        prep_all(1 - par, lp + par)

            def pair(lp, c):
                phase(0, lp, xa_ref, xb_ref)
                phase(1, lp, xb_ref, xa_ref)
                return c
            jax.lax.fori_loop(0, L // 2, pair, 0)
            o_ref[...] = xa_ref[...].astype(o_ref.dtype)

        @pl.when(pl.program_id(0) > 0)
        def _rest():
            def tile(t, c):
                rows = pl.ds(pl.multiple_of(t * tm, tm), tm)
                x0t, ot = x0_ref.at[rows], o_ref.at[rows]
                X0 = {k: blk(x0t, *k)[...].astype(f32) for k in BLOCKS}
                X = X0
                for l in range(L):
                    new = {}
                    def emit(q, s, y):
                        if l == L - 1:
                            blk(ot, q, s)[...] = y.astype(o_ref.dtype)
                        else:
                            new[q, s] = y
                    layer(l % 2, lambda q, s: X[q, s], lambda q, s: X0[q, s], wload(l % 2, l // 2),
                          lambda q, s: b_ref[l // 2, l % 2:l % 2 + 1, rc(q, s)[1] * h:(rc(q, s)[1] + 1) * h].astype(f32), emit)
                    X = new
                return c
            jax.lax.fori_loop(0, T, tile, 0)

    @jax.jit
    def f(x0, ws, bs):
        B, D = x0.shape
        L = ws.shape[0]
        sshape = (L // 2 + 1, 49, D // 8, D // 4) if u32 else (L // 2 + 1, 49, D // 4, D // 4)
        sdt = jnp.uint32 if u32 else bf16
        return pl.pallas_call(
            kern,
            grid=(B // (tm * T),),
            in_specs=[pl.BlockSpec((tm * T, D), lambda i: (i, 0)),
                      pl.BlockSpec(memory_space=pl.ANY),
                      pl.BlockSpec((L // 2, 2, D), lambda i: (0, 0, 0), pipeline_mode=pl.Buffered(1))],
            out_specs=pl.BlockSpec((tm * T, D), lambda i: (i, 0)),
            out_shape=jax.ShapeDtypeStruct((B, D), x0.dtype),
            scratch_shapes=[pltpu.VMEM(sshape, sdt), pltpu.VMEM(sshape, sdt), pltpu.VMEM((2, D, D), bf16),
                            pltpu.VMEM((tm * T, D), f32), pltpu.VMEM((tm * T, D), f32), pltpu.SemaphoreType.DMA((2,))],
            compiler_params=pltpu.CompilerParams(dimension_semantics=("arbitrary",), vmem_limit_bytes=vmem * 1024 * 1024, flags=flags),
        )(x0, ws, bs.reshape(L // 2, 2, D))
    return f


_f = build(T=1, overlap=False)


@jax.jit
def pallas_standalone__cross_network_dcn__recsys_kernel(x0, ws, bs):
    return _f(x0, ws, bs)
```

```python
import jax
import jax.numpy as jnp
import jax.experimental.pallas as pl
import jax.experimental.pallas.tpu as pltpu

f32 = jnp.float32
bf16 = jnp.bfloat16

TILE = 256
TILES = 2
PREP_ROWS = 16

A_TERMS = {1: ((1, 0), (1, 3)), 2: ((1, 2), (1, 3)), 3: ((1, 0),), 4: ((1, 3),),
           5: ((1, 0), (1, 1)), 6: ((1, 2), (-1, 0)), 7: ((1, 1), (-1, 3))}
B_TERMS = {1: ((1, 0), (1, 3)), 2: ((1, 0),), 3: ((1, 1), (-1, 3)), 4: ((1, 2), (-1, 0)),
           5: ((1, 3),), 6: ((1, 0), (1, 1)), 7: ((1, 2), (1, 3))}
C_TERMS = {1: ((1, 0), (1, 3)), 2: ((1, 2), (-1, 3)), 3: ((1, 1), (1, 3)), 4: ((1, 0), (1, 2)),
           5: ((-1, 0), (1, 1)), 6: ((1, 3),), 7: ((1, 0),)}
C_COUNT = (4, 2, 2, 4)
OUTER = ((3, 5, 6, 1, 2, 4, 7), (4, 2, 7, 1, 5, 3, 6))
INNER = (7, 4, 2, 1, 6, 3, 5)
BLOCKS = tuple((q, s) for q in range(4) for s in range(4))


def _row_col(q, s):
    return (q // 2) * 2 + s // 2, (q % 2) * 2 + s % 2


def _addsub(u, v, sign):
    return u + v if sign > 0 else u - v


def _combine(terms, get):
    u = get(terms[0][1])
    return u if len(terms) == 1 else _addsub(u, get(terms[1][1]), terms[1][0])


def _join(a, b):
    (sa, va), (sb, vb) = a, b
    if sa < 0 < sb:
        return 1, vb - va
    return sa, _addsub(va, vb, sa * sb)


def _lhs(m1, m2, x):
    t1, t2 = A_TERMS[m1], A_TERMS[m2]
    if len(t1) == 1 or len(t2) == 1:
        return _combine(t2, lambda s: _combine(t1, lambda q: x(q, s)))
    (_, q0), (g1, q1) = t1
    (_, s0), (g2, s1) = t2
    diag = _join((1, x(q0, s0)), (g1 * g2, x(q1, s1)))
    anti = _join((g1, x(q1, s0)), (g2, x(q0, s1)))
    return _join(diag, anti)[1]


def _layer(parity, x, x0, w, bias, emit):
    parts = {k: [] for k in BLOCKS}
    todo = {(q, s): C_COUNT[q] for q, s in BLOCKS}
    for m1 in OUTER[parity]:
        acc = [None] * 4
        left = list(C_COUNT)
        for m2 in INNER:
            p = jnp.dot(_lhs(m1, m2, x).astype(bf16), w((m1 - 1) * 7 + m2 - 1),
                        preferred_element_type=f32)
            for sign, s in C_TERMS[m2]:
                acc[s] = (sign, p) if acc[s] is None else _join(acc[s], (sign, p))
                left[s] -= 1
                if left[s]:
                    continue
                for sign1, q in C_TERMS[m1]:
                    parts[q, s].append((sign1 * acc[s][0], acc[s][1]))
                    todo[q, s] -= 1
                    if todo[q, s] and m1 == 1:
                        continue
                    total = parts[q, s][0]
                    for part in parts[q, s][1:]:
                        total = _join(total, part)
                    parts[q, s] = [total]
                    if not todo[q, s]:
                        proj = _join(total, (1, bias(q, s)))[1]
                        emit(q, s, x0(q, s) * proj + x(q, s))


def _kernel(x0_ref, w_hbm, b_ref, o_ref, s_ref, wbuf, xa_ref, xb_ref, bf_ref, sem):
    L, D, _ = w_hbm.shape
    h = D // 4
    qm = TILE // 4

    def block(ref, q, s):
        r, c = _row_col(q, s)
        return ref.at[r * qm:(r + 1) * qm, c * h:(c + 1) * h]

    def weights(l):
        return lambda k: pltpu.bitcast(s_ref[l, k], bf16)

    def bias(l):
        return lambda q, s: bf_ref[pl.ds(l, 1), pl.ds(_row_col(q, s)[1] * h, h)]

    def w_copy(l, slot):
        return pltpu.make_async_copy(w_hbm.at[l], wbuf.at[slot], sem.at[slot])

    def prepare(l, slot):
        def body(i, carry):
            r0 = pl.multiple_of(i * PREP_ROWS, PREP_ROWS)
            words = pl.ds(pl.multiple_of(i * (PREP_ROWS // 2), PREP_ROWS // 2), PREP_ROWS // 2)
            b = {}
            for q, s in BLOCKS:
                r, c = _row_col(q, s)
                b[q, s] = wbuf[slot, pl.ds(r * h + r0, PREP_ROWS), c * h:(c + 1) * h].astype(f32)
            for m1 in range(1, 8):
                sub = [_combine(B_TERMS[m1], lambda q: b[q, s]) for s in range(4)]
                for m2 in range(1, 8):
                    v = _combine(B_TERMS[m2], lambda s: sub[s]).astype(bf16)
                    s_ref[l, (m1 - 1) * 7 + m2 - 1, words, :] = pltpu.bitcast(v, jnp.uint32)
            return carry
        jax.lax.fori_loop(0, h // PREP_ROWS, body, 0)

    @pl.when(pl.program_id(0) == 0)
    def _first_step():
        w_copy(0, 0).start()
        xa_ref[...] = x0_ref[...].astype(f32)
        bf_ref[...] = b_ref[...].astype(f32)
        w_copy(0, 0).wait()
        w_copy(1, 1).start()
        prepare(0, 0)

        def phase(l, parity, src, dst):
            @pl.when(l + 2 < L)
            def _():
                w_copy(l + 2, parity).start()

            def tile(t, carry):
                rows = pl.ds(pl.multiple_of(t * TILE, TILE), TILE)
                x0_t, src_t, dst_t = x0_ref.at[rows], src.at[rows], dst.at[rows]

                def emit(q, s, y):
                    block(dst_t, q, s)[...] = y

                _layer(parity, lambda q, s: block(src_t, q, s)[...],
                       lambda q, s: block(x0_t, q, s)[...].astype(f32),
                       weights(l), bias(l), emit)
                return carry
            jax.lax.fori_loop(0, TILES, tile, 0)

            @pl.when(l + 1 < L)
            def _():
                w_copy(l + 1, 1 - parity).wait()
                prepare(l + 1, 1 - parity)

        def two_layers(i, carry):
            phase(2 * i, 0, xa_ref, xb_ref)
            phase(2 * i + 1, 1, xb_ref, xa_ref)
            return carry
        jax.lax.fori_loop(0, L // 2, two_layers, 0)
        o_ref[...] = xa_ref[...].astype(o_ref.dtype)

    @pl.when(pl.program_id(0) > 0)
    def _other_steps():
        for t in range(TILES):
            rows = pl.ds(t * TILE, TILE)
            x0_t, o_t = x0_ref.at[rows], o_ref.at[rows]
            x0 = {k: block(x0_t, *k)[...].astype(f32) for k in BLOCKS}
            x = x0
            for l in range(L):
                new = {}

                def emit(q, s, y):
                    if l == L - 1:
                        block(o_t, q, s)[...] = y.astype(o_ref.dtype)
                    else:
                        new[q, s] = y

                _layer(l % 2, lambda q, s: x[q, s], lambda q, s: x0[q, s],
                       weights(l), bias(l), emit)
                x = new


@jax.jit
def pallas_standalone__cross_network_dcn__recsys_kernel(
    x0: jax.Array,
    ws: jax.Array,
    bs: jax.Array,
):
    B, D = x0.shape
    L = ws.shape[0]
    rows = TILE * TILES
    assert B % rows == 0 and D % 512 == 0 and L % 2 == 0 and ws.dtype == bf16
    return pl.pallas_call(
        _kernel,
        grid=(B // rows,),
        in_specs=[
            pl.BlockSpec((rows, D), lambda i: (i, 0)),
            pl.BlockSpec(memory_space=pl.ANY),
            pl.BlockSpec((L, D), lambda i: (0, 0)),
        ],
        out_specs=pl.BlockSpec((rows, D), lambda i: (i, 0)),
        out_shape=jax.ShapeDtypeStruct((B, D), x0.dtype),
        scratch_shapes=[
            pltpu.VMEM((L, 49, D // 8, D // 4), jnp.uint32),
            pltpu.VMEM((2, D, D), bf16),
            pltpu.VMEM((rows, D), f32),
            pltpu.VMEM((rows, D), f32),
            pltpu.VMEM((L, D), f32),
            pltpu.SemaphoreType.DMA((2,)),
        ],
        compiler_params=pltpu.CompilerParams(
            dimension_semantics=("arbitrary",),
            vmem_limit_bytes=100 * 1024 * 1024,
        ),
    )(x0, ws, bs)
```
